```python
import os as _os
_os.environ.setdefault("JAX_PLATFORMS", "cpu")
import jax
import jax.numpy as jnp

def _softmax(x, axis=-1):
    return jax.nn.softmax(x, axis=axis)
def _gelu(x):
    return jax.nn.gelu(x, approximate=True)
def _silu(x):
    return jax.nn.silu(x)
def _sigmoid(x):
    return jax.nn.sigmoid(x)
def _layernorm(x, axis=-1, eps=1e-5):
    m = jnp.mean(x, axis=axis, keepdims=True)
    v = jnp.var(x, axis=axis, keepdims=True)
    return (x - m) / jnp.sqrt(v + eps)
def _scatter_add(tgt, idx, src, axis=0):
    return tgt.at[idx].add(src)
def _segment_sum(src, seg, n):
    return jax.ops.segment_sum(src, seg, n)
class _Rng:
    def __init__(self, key):
        self._k = key
    def _next(self):
        self._k, sub = jax.random.split(self._k)
        return sub
    def normal(self, shape):
        return jax.random.normal(self._next(), shape, dtype=jnp.bfloat16)
    def randint(self, lo, hi, shape):
        return jax.random.randint(self._next(), shape, lo, hi, dtype=jnp.int32)
    def uniform(self, shape, lo=0.0, hi=1.0):
        return jax.random.uniform(self._next(), shape, jnp.bfloat16, lo, hi)
    def permutation(self, n):
        return jax.random.permutation(self._next(), n)


kernel_name = 'concat_heads__gqa_block_cached__mha_block_cached__near_ridge'

def setup_inputs():
    _rng = _Rng(jax.random.key(int.from_bytes(__import__("os").urandom(4), "little")))
    _w = (lambda a: (lambda t: t.astype(jnp.bfloat16) if jnp.issubdtype(t.dtype, jnp.floating) else t)(jnp.asarray(a)))
    def _A_setup():
        B, Sq, D = 8, 112, 448
        Hq, Hkv, Sk, Dh = 16, 8, 512, 256
        assert Hq % Hkv == 0, (Hq, Hkv)
        return {
            "x": _w((lambda *s: _rng.normal(s) * 0.8)(B, Sq, D)),
            "k_cache": _w((lambda *s: _rng.normal(s) * 0.8)(B, Hkv, Sk, Dh)),
            "v_cache": _w((lambda *s: _rng.normal(s) * 0.05)(B, Hkv, Sk, Dh)),
            "wq": _w((lambda *s: _rng.normal(s) * 0.8)(D, Hq * Dh) * (D ** -0.5)),
            "wo": _w((lambda *s: _rng.normal(s) * 0.05)(Hq * Dh, D) * ((Hq * Dh) ** -0.5)),
        }
    _A_in = _A_setup()

    def _B_setup():
        B, Sq, D = 8, 112, 448
        H, Sk, Dh = 16, 512, 256
        return {
            "x": _w((lambda *s: _rng.normal(s) * 0.8)(B, Sq, D)),
            "k_cache": _w((lambda *s: _rng.normal(s) * 0.8)(B, H, Sk, Dh)),
            "v_cache": _w((lambda *s: _rng.normal(s) * 0.05)(B, H, Sk, Dh)),
            "wq": _w((lambda *s: _rng.normal(s) * 0.8)(D, H * Dh) * (D ** -0.5)),
            "wo": _w((lambda *s: _rng.normal(s) * 0.05)(H * Dh, D) * ((H * Dh) ** -0.5)),
        }
    _B_in = _B_setup()

    return {
        "A_x": _A_in["x"],
        "A_k_cache": _A_in["k_cache"],
        "A_v_cache": _A_in["v_cache"],
        "A_wq": _A_in["wq"],
        "A_wo": _A_in["wo"],
        "B_x": _B_in["x"],
        "B_k_cache": _B_in["k_cache"],
        "B_v_cache": _B_in["v_cache"],
        "B_wq": _B_in["wq"],
        "B_wo": _B_in["wo"],
    }

def reference(A_x, A_k_cache, A_v_cache, A_wq, A_wo, B_x, B_k_cache, B_v_cache, B_wq, B_wo):
    def _A_ref(x, k_cache, v_cache, wq, wo):
        B, Sq, D = x.shape
        Hq, Dh = 16, 256
        Hkv = k_cache.shape[1]
        rep = Hq // Hkv
        q = (lambda x, *d: x.transpose(*d))((x @ wq).reshape(B, Sq, Hq, Dh), 0, 2, 1, 3)
        k = jnp.repeat(k_cache, rep, axis=1)
        v = jnp.repeat(v_cache, rep, axis=1)
        scores = jnp.einsum("bhqd,bhkd->bhqk", q, k) * (Dh ** -0.5)
        p = _softmax(scores, axis=-1)
        o = jnp.einsum("bhqk,bhkd->bhqd", p, v)
        return (lambda x, *d: x.transpose(*d))(o, 0, 2, 1, 3).reshape(B, Sq, Hq * Dh) @ wo

    def _B_ref(x, k_cache, v_cache, wq, wo):
        B, Sq, D = x.shape
        H, Dh = 16, 256
        q = (lambda x, *d: x.transpose(*d))((x @ wq).reshape(B, Sq, H, Dh), 0, 2, 1, 3)
        scores = jnp.einsum("bhqd,bhkd->bhqk", q, k_cache) * (Dh ** -0.5)
        p = _softmax(scores, axis=-1)
        o = jnp.einsum("bhqk,bhkd->bhqd", p, v_cache)
        return (lambda x, *d: x.transpose(*d))(o, 0, 2, 1, 3).reshape(B, Sq, H * Dh) @ wo

    a = _A_ref(A_x, A_k_cache, A_v_cache, A_wq, A_wo)
    b = _B_ref(B_x, B_k_cache, B_v_cache, B_wq, B_wo)
    return jnp.concatenate([a, b], axis=-1)
```

```python
import math

import jax
import jax.numpy as jnp
from jax import lax
from jax.experimental import pallas as pl
from jax.experimental.pallas import tpu as pltpu

B, SQ, D = 8, 112, 448
H, SK, DH = 16, 512, 256
G = H // 2
GW = 2 * DH
T = B * SQ
TT = 128
NT = T // TT
BF = jnp.bfloat16
F32 = jnp.float32
_NT_DIMS = (((1,), (1,)), ((), ()))
_C = (DH ** -0.5) * math.log2(math.e)
CHUNKS = (0, 9, 13)
NCH = len(CHUNKS)
U3 = 3
ORDER2 = (('s', 2), ('f', 0), ('x', 1), ('v', 0))
ORDER4 = (('w', 3), ('x', 1), ('v', 0), ('s', 3), ('l', 1), ('f', 0))
N2 = 14
N4 = 27
N5 = (10, 8, 10)
LATE = 6
LAG = 3
SPLIT3 = 7
BULK = 1
SMALL = 0


def _dot_nt(a, b):
    return lax.dot_general(a, b, _NT_DIMS, preferred_element_type=F32)


def _softmax(s):
    m = jnp.max(s, axis=-1, keepdims=True)
    e = jnp.exp2((s - m) * _C)
    l = jnp.sum(e, axis=-1, keepdims=True)
    return (e * (1.0 / l)).astype(BF)


def _heads(h0, h1):
    return pl.ds(h0 * SK, (h1 - h0) * SK)


def _split(r0, r1, n):
    cuts = [r0 + (r1 - r0) // 16 * i // n * 16 for i in range(n + 1)]
    return [pl.ds(a, b - a) for a, b in zip(cuts, cuts[1:])]


def _kernel(xa_h, ka_h, va_h, wqa_h, woa_h, xb_h, kb_h, vb_h, wqb_h, wob_h, out_h,
            x_v, wq_v, wo_v, kva_v, kvb_v, q_v, o_v, acc_v, part_v, out_v,
            x_sem, wq_sem, wo_sem, a_sem, kb_sem, vb_sem, out_sem):
    cp = pltpu.make_async_copy

    def x_cp(br):
        return cp((xa_h, xb_h)[br], x_v.at[br], x_sem.at[br])

    def wqa_cp(g):
        return cp(wqa_h.at[:, pl.ds(pl.multiple_of(g * GW, GW), GW)], wq_v.at[g], wq_sem.at[g])

    def kb_cp(b, h0, h1, sem):
        return cp(kb_h.at[b, _heads(h0, h1)], kvb_v.at[b, _heads(h0, h1)], kb_sem.at[sem])

    def kb_late(b, c):
        return kb_cp(b, CHUNKS[c], (CHUNKS + (H,))[c + 1], LATE + (b - LATE) * NCH + c)

    def out_cp(i):
        r0, r1 = ((0, T - TT), (T - TT, T))[i]
        return cp(out_v.at[pl.ds(r0, r1 - r0)], out_h.at[pl.ds(r0, r1 - r0)], out_sem.at[i])

    wqa_cp(0).start(priority=BULK)
    x_cp(0).start(priority=BULK)

    def i1(g, c):
        wqa_cp(g).start(priority=BULK)
        return c
    lax.fori_loop(1, G, i1, 0)
    x_cp(1).start(priority=BULK)
    cp(ka_h.at[0], kva_v.at[0], a_sem.at[0]).start(priority=BULK)
    cp(va_h.at[0], kva_v.at[2], a_sem.at[1]).start(priority=BULK)

    def i2(i, c):
        @pl.when(i == 0)
        def _():
            cp(woa_h, wo_v.at[0], wo_sem.at[0]).start(priority=BULK)
            cp(vb_h.at[0], kvb_v.at[B], vb_sem.at[0]).start(priority=BULK)
        kb_cp(i, 0, H, i).start(priority=BULK)
        return c
    lax.fori_loop(0, LATE, i2, 0)

    def i3(i, c):
        for j in range(NCH):
            @pl.when(i % NCH == j)
            def _():
                kb_late(LATE + i // NCH, j).start(priority=BULK)
        return c
    lax.fori_loop(0, (B - LATE) * NCH, i3, 0)
    part_v[...] = jnp.zeros((D, TT), F32)

    x_cp(0).wait()

    def p1(g, c):
        wqa_cp(g).wait()
        cols = pl.ds(pl.multiple_of(g * GW, GW), GW)
        for j in range(2 * B):
            b, u = j // 2, j % 2
            q = jnp.dot(x_v[0, b * SQ:(b + 1) * SQ], wq_v[g, :, u * DH:(u + 1) * DH], preferred_element_type=F32)
            q_v[0][g, b, u * SQ:(u + 1) * SQ, :] = q.astype(BF)
            if j < 14:
                rows = pl.ds(j * 32, 32)
                cp(wqb_h.at[rows, cols], wq_v.at[G + g, rows], wq_sem.at[G + g]).start(priority=SMALL)
        return c
    lax.fori_loop(0, G, p1, 0)

    x_cp(1).wait()

    def p2(b, c):
        cur, nxt = b % 2, (b + 1) % 2
        cp(wq_v.at[G + b], wq_v.at[G + b], wq_sem.at[G + b]).wait()
        cp(kva_v.at[cur], kva_v.at[cur], a_sem.at[0]).wait()
        cp(kva_v.at[2 + cur], kva_v.at[2 + cur], a_sem.at[1]).wait()
        row = pl.multiple_of(b * SQ, 16)
        s, p = {}, {}
        todo = [(kv, rows) for kv in range(2) for rows in _split(0, G * SK, N2)]
        for i in range(-4, H + 4):
            for op, off in ORDER2:
                h = i + off
                if not 0 <= h < H:
                    continue
                g, u = h // 2, h % 2
                if op == 's':
                    s[h] = _dot_nt(q_v[0][g, b, u * SQ:(u + 1) * SQ], kva_v[cur, _heads(g, g + 1)])
                elif op == 'x':
                    p[h] = _softmax(s[h])
                elif op == 'f':
                    q = jnp.dot(x_v[1, g * SQ:(g + 1) * SQ], wq_v[G + b, :, u * DH:(u + 1) * DH],
                                preferred_element_type=F32)
                    q_v[1][b, g, u * SQ:(u + 1) * SQ, :] = q.astype(BF)
                elif op == 'v':
                    o = jnp.dot(p[h], kva_v[2 + cur, _heads(g, g + 1)], preferred_element_type=F32)
                    o_v[g][pl.ds(row, SQ), u * DH:(u + 1) * DH] = o.astype(BF)
                if op in 'sv' and todo:
                    kv, rows = todo.pop(0)

                    @pl.when(b + 1 < B)
                    def _():
                        cp((ka_h, va_h)[kv].at[b + 1, rows], kva_v.at[2 * kv + nxt, rows],
                           a_sem.at[kv]).start(priority=SMALL)
        assert not todo
        return c
    lax.fori_loop(0, B, p2, 0)

    def oproj_chunk(br, t, g):
        row = pl.multiple_of(t * TT, TT)
        return _dot_nt(wo_v[br, :, g * GW:(g + 1) * GW], o_v[g][pl.ds(row, TT), :])

    cp(woa_h, wo_v.at[0], wo_sem.at[0]).wait()
    n3 = (NT - 1) // U3
    pieces = D // 16 // n3

    def p3(i, c):
        todo = [(j, c0, c1) for j in range(pieces)
                for c0, c1 in (((0, H * DH // 2), (H * DH // 2, H * DH)) if j < SPLIT3 else ((0, H * DH),))]
        done = None
        for u in range(U3):
            t = i * U3 + u
            acc = None
            for g in range(G):
                part = oproj_chunk(0, t, g)
                acc = part if acc is None else acc + part
                if todo and g > 0:
                    j, c0, c1 = todo.pop(0)
                    rows, cols = pl.ds(pl.multiple_of((i * pieces + j) * 16, 16), 16), pl.ds(c0, c1 - c0)
                    cp(wob_h.at[rows, cols], wo_v.at[1, rows, cols], wo_sem.at[1]).start(priority=SMALL)
                if done is not None:
                    acc_v[t - 1] = done
                    done = None
            done = acc
        acc_v[i * U3 + U3 - 1] = done
        assert not todo
        return c
    lax.fori_loop(0, n3, p3, 0)


    vcut = (0,) + tuple(h - LAG for h in CHUNKS[1:]) + (H,)

    def p4(b, late):
        row = pl.multiple_of(T + b * SQ, 16)
        cur, nxt = b % 2, (b + 1) % 2
        if late:
            todo = [(0, j, r) for j in range(1, NCH) for r in _split(vcut[j] * SK, vcut[j + 1] * SK, N5[j])]
            todo += [(1, 0, r) for r in _split(0, vcut[1] * SK, N5[0])]
        else:
            @pl.when(b == 1)
            def _():
                cp(wob_h, wo_v.at[1], wo_sem.at[1]).wait()
            kb_cp(b, 0, H, b).wait()
            cp(kvb_v.at[B + cur], kvb_v.at[B + cur], vb_sem.at[0]).wait()
            todo = [(1, 0, r) for r in _split(0, H * SK, N4)]
        s, p = {}, {}
        acc = None
        for i in range(-4, H + 6):
            for op, off in ORDER4:
                h = i + off
                if not 0 <= h < H:
                    continue
                if op == 'w':
                    if late and h in CHUNKS:
                        j = CHUNKS.index(h)
                        assert j == 0 or todo[0][0] or todo[0][1] > j
                        kb_late(b, j).wait()
                        vs = kvb_v.at[B + cur, _heads(vcut[j], vcut[j + 1])]

                        @pl.when(b > LATE)
                        def _():
                            cp(vs, vs, vb_sem.at[j]).wait()
                        if j == NCH - 1:
                            def send(_, c2):
                                out_cp(0).start()
                                return c2
                            lax.fori_loop(0, jnp.where(b == B - 1, 1, 0), send, 0)
                elif op == 's':
                    s[h] = _dot_nt(q_v[1][h // 2, b, (h % 2) * SQ:(h % 2 + 1) * SQ], kvb_v[b, _heads(h, h + 1)])
                elif op == 'x':
                    p[h] = _softmax(s[h])
                elif op == 'v':
                    o = jnp.dot(p[h], kvb_v[B + cur, _heads(h, h + 1)], preferred_element_type=F32).astype(BF)
                    o_v[h // 2][pl.ds(row, SQ), (h % 2) * DH:(h % 2 + 1) * DH] = o
                elif op == 'l' and h == 0:
                    done = part_v[...] + oproj_chunk(jnp.where(b >= 2, 1, 0), NT - 2 + b, G - 1)
                    t = jnp.maximum(b - 2, 0)
                    full = jnp.concatenate([acc_v[t], done], axis=0)
                    out_v[pl.ds(pl.multiple_of(t * TT, TT), TT), :] = full.T.astype(BF)
                    acc_v[jnp.where(b == 1, NT - 1, NT)] = done
                elif op == 'f' and h % 2 == 0 and h > 0:
                    part = oproj_chunk(jnp.minimum(b, 1), NT - 1 + b, h // 2 - 1)
                    acc = part if acc is None else acc + part
                if op in 'sv' and todo:
                    ahead, sem, rows = todo.pop(0)
                    piece = cp(vb_h.at[jnp.minimum(b + ahead, B - 1), rows], kvb_v.at[B + (cur, nxt)[ahead], rows], vb_sem.at[sem])
                    if late:
                        pl.when(b + 1 < B if ahead else b > LATE)(lambda: piece.start(priority=SMALL))
                    else:
                        piece.start(priority=SMALL)
        assert not todo
        part_v[...] = acc

    def p4a(b, c):
        p4(b, False)
        return c
    lax.fori_loop(0, LATE, p4a, 0)
    cp(kvb_v.at[B + LATE % 2], kvb_v.at[B + LATE % 2], vb_sem.at[0]).wait()

    def p4b(b, c):
        p4(b, True)
        return c
    lax.fori_loop(LATE, B, p4b, 0)

    head = jnp.concatenate([acc_v[NT - 1], part_v[...]], axis=0).T
    pad = D % TT
    w_last = jnp.concatenate([jnp.zeros((pad, GW), BF), wo_v[1, :, (G - 1) * GW:G * GW]], axis=0)
    last = _dot_nt(o_v[G - 1][2 * T - TT:2 * T, :], w_last)
    out_v[T - TT:T, 0:D - pad] = head[:, 0:D - pad].astype(BF)
    out_v[T - TT:T, D - pad:2 * D] = (head[:, D - pad:2 * D] + last).astype(BF)
    out_cp(1).start()
    out_cp(0).wait()
    out_cp(1).wait()


@jax.jit
def pallas_concat_heads__gqa_block_cached__mha_block_cached__near_ridge_kernel(
        A_x, A_k_cache, A_v_cache, A_wq, A_wo, B_x, B_k_cache, B_v_cache, B_wq, B_wo):
    out = pl.pallas_call(
        _kernel,
        out_shape=jax.ShapeDtypeStruct((T, 2 * D), BF),
        in_specs=[pl.BlockSpec(memory_space=pl.ANY)] * 10,
        out_specs=pl.BlockSpec(memory_space=pl.ANY),
        scratch_shapes=[
            pltpu.VMEM((2, T, D), BF),
            pltpu.VMEM((2 * G, D, GW), BF),
            pltpu.VMEM((2, D, H * DH), BF),
            pltpu.VMEM((4, G * SK, DH), BF),
            pltpu.VMEM((B + 2, H * SK, DH), BF),
            [pltpu.VMEM((G, B, 2 * SQ, DH), BF)] * 2,
            [pltpu.VMEM((2 * T, GW), BF)] * G,
            pltpu.VMEM((NT + 1, D, TT), F32),
            pltpu.VMEM((D, TT), F32),
            pltpu.VMEM((T, 2 * D), BF),
            pltpu.SemaphoreType.DMA((2,)),
            pltpu.SemaphoreType.DMA((2 * G,)),
            pltpu.SemaphoreType.DMA((2,)),
            pltpu.SemaphoreType.DMA((2,)),
            pltpu.SemaphoreType.DMA((LATE + (B - LATE) * NCH,)),
            pltpu.SemaphoreType.DMA((NCH,)),
            pltpu.SemaphoreType.DMA((2,)),
        ],
        compiler_params=pltpu.CompilerParams(vmem_limit_bytes=110 * 1024 * 1024, disable_bounds_checks=True, disable_semaphore_checks=True),
    )(A_x.reshape(T, D), A_k_cache.reshape(B, G * SK, DH), A_v_cache.reshape(B, G * SK, DH), A_wq, A_wo.T,
      B_x.reshape(T, D), B_k_cache.reshape(B, H * SK, DH), B_v_cache.reshape(B, H * SK, DH), B_wq, B_wo.T)
    return out.reshape(B, SQ, 2 * D)
```

```python
import math

import jax
import jax.numpy as jnp
from jax import lax
from jax.experimental import pallas as pl
from jax.experimental.pallas import tpu as pltpu

B, SQ, D = 8, 112, 448
H, SK, DH = 16, 512, 256
G = H // 2
GW = 2 * DH
T = B * SQ
TT = 128
NT = T // TT
PAD = D % TT
HALF = D // 2
BF = jnp.bfloat16
F32 = jnp.float32
SCALE_LOG2E = DH ** -0.5 * math.log2(math.e)

BULK, SMALL = 1, 0
WQA, WQB, WOA, WOB = (i * G for i in range(4))
XCUT = (0, 2, 5, 8)
U1, U3 = 3, 3
LAG = 3
LATE = 6
VT = 4
KCUT = (0, 9, 14, H)
VCUT = (VT,) + tuple(h - LAG for h in KCUT[1:-1]) + (H,)
NCH = len(KCUT) - 1
N2, NW, N3, N4, N5 = 56, 14, 9, 58, 56


def _dot(a, b):
    return jnp.dot(a, b, preferred_element_type=F32)


def _dot_nt(a, b):
    return lax.dot_general(a, b, (((1,), (1,)), ((), ())), preferred_element_type=F32)


def _softmax(s):
    m = jnp.max(s, axis=-1, keepdims=True)
    e = jnp.exp2((s - m) * SCALE_LOG2E)
    return (e * (1.0 / jnp.sum(e, axis=-1, keepdims=True))).astype(BF)


def _ds(start, size, align):
    return pl.ds(start if isinstance(start, int) else pl.multiple_of(start, align), size)


def _heads(h0, h1):
    return pl.ds(h0 * SK, (h1 - h0) * SK)


def _tile(t):
    return _ds(t * TT, TT, TT)


def _split(rows, n):
    cuts = [rows // 16 * i // n * 16 for i in range(n + 1)]
    return [pl.ds(a, b - a) for a, b in zip(cuts, cuts[1:])]


def _kernel(xa_h, ka_h, va_h, wqa_h, woa_h, xb_h, kb_h, vb_h, wqb_h, wob_h, out_h,
            x_v, w_v, kv_v, q_v, o_v, acc_v, part_v, out_v,
            x_sem, wq_sem, wo_sem, ka_sem, va_sem, kb_sem, vb_sem, out_sem):
    copy = pltpu.make_async_copy

    def wait_filled(buf, sem):
        copy(buf, buf, sem).wait()

    def w_cp(src, base, g, rows, sem):
        return copy(src.at[rows, _ds(g * GW, GW, GW)], w_v.at[base + g, rows], sem)

    def wqa_cp(g):
        return w_cp(wqa_h, WQA, g, slice(None), wq_sem.at[g])

    def wq0_cp(u):
        cols = pl.ds(u * DH, DH)
        return copy(wqa_h.at[:, cols], w_v.at[WQA, :, cols], x_sem.at[len(XCUT) + u])

    def xa_cp(j):
        rows = pl.ds(XCUT[j] * SQ, (XCUT[j + 1] - XCUT[j]) * SQ)
        return copy(xa_h.at[rows], x_v.at[0, rows], x_sem.at[j])

    def ka_buf(b, start, size):
        return kv_v.at[B + 2 + b // 2, _ds(b % 2 * G * SK + start, size, 16)]

    def va_buf(b, start, size):
        return kv_v.at[B + 6, _ds(b % 2 * G * SK + start, size, 16)]

    def ka_cp(b):
        return copy(ka_h.at[b], ka_buf(b, 0, G * SK), ka_sem.at[b])

    def vb_cp(b, rows, sem):
        return copy(vb_h.at[b, rows], kv_v.at[B + b, rows], sem)

    def vb_first(b, rows):
        return vb_cp(b, rows, vb_sem.at[b % 2])

    def kvb_early(b):
        return [copy(kb_h.at[b], kv_v.at[b], kb_sem.at[b]),
                vb_cp(b, _heads(VT, H), kb_sem.at[b])]

    def kvb_late(b, j):
        sem = kb_sem.at[LATE + (b - LATE) * NCH + j]
        rows = _heads(KCUT[j], KCUT[j + 1])
        return [copy(kb_h.at[b, rows], kv_v.at[b, rows], sem),
                vb_cp(b, _heads(VCUT[j], VCUT[j + 1]), sem)]

    def out_cp(i):
        idx = ((pl.ds(0, T - TT), slice(None)),
               (_tile(NT - 1), pl.ds(0, D - PAD)),
               (_tile(NT - 1), pl.ds(D - PAD, 2 * TT)),
               (_tile(NT - 1), pl.ds(D - PAD + 2 * TT, 2 * TT)))[i]
        return copy(out_v.at[idx], out_h.at[idx], out_sem.at[i])

    def start_in_order(lo, hi, copies):
        def trip(i, carry):
            for c in copies(i):
                c.start(priority=BULK)
            return carry
        lax.fori_loop(lo, hi, trip, 0)

    def scores(q, k_ref, trickle):
        parts = []
        for j in range(2):
            parts.append(_dot_nt(q, k_ref(j * SK // 2, SK // 2)))
            trickle()
        return jnp.concatenate(parts, axis=1)

    def store_pv(p, v_ref, h, row, trickle):
        for j in range(2):
            o = _dot(p, v_ref(pl.ds(j * DH // 2, DH // 2)))
            o_v[h // 2][pl.ds(row, SQ), pl.ds(h % 2 * DH + j * DH // 2, DH // 2)] = o.astype(BF)
            trickle()

    def qproj(br, g, b, u):
        q = _dot(x_v[br, b * SQ:(b + 1) * SQ], w_v[br * G + g, :, u * DH:(u + 1) * DH])
        q_v[br][g, b, u * SQ:(u + 1) * SQ, :] = q.astype(BF)

    def oproj(w0, t, g, rows=slice(None)):
        return _dot_nt(w_v[w0 + g, rows, :], o_v[g][_tile(t), :])

    wq0_cp(0).start(priority=BULK)
    xa_cp(0).start(priority=BULK)

    def start_xa(i, carry):
        pl.when(i == 0)(lambda: wq0_cp(1).start(priority=BULK))
        for j in range(1, len(XCUT) - 1):
            pl.when(i == j)(lambda: xa_cp(j).start(priority=BULK))
        return carry
    lax.fori_loop(0, len(XCUT) - 1, start_xa, 0)
    wqa_cp(1).start(priority=BULK)
    start_in_order(4, G, lambda g: [wqa_cp(g)])
    xb_cp = copy(xb_h, x_v.at[1], x_sem.at[len(XCUT) - 1])
    xb_cp.start(priority=BULK)
    copy(va_h.at[0], va_buf(0, 0, G * SK), va_sem).start(priority=BULK)
    start_in_order(0, B, lambda b: [ka_cp(b)])
    start_in_order(0, 2, kvb_early)

    xa_cp(0).wait()
    for u in range(2):
        wq0_cp(u).wait()
        for b in range(XCUT[1]):
            qproj(0, 0, b, u)
    for j in range(1, len(XCUT) - 1):
        xa_cp(j).wait()
        units = [(0, b) for b in range(XCUT[j], XCUT[j + 1])]
        if j == len(XCUT) - 2:
            wqa_cp(1).wait()
            units += [(1, b) for b in range(B)]
        todo = [(g, rows) for g in (2, 3) for rows in _split(D, 8)] if j == len(XCUT) - 2 else []
        for g, b in units:
            for u in range(2):
                qproj(0, g, b, u)
                if todo:
                    n, rows = todo.pop(0)
                    w_cp(wqa_h, WQA, n, rows, wq_sem.at[n]).start(priority=SMALL)

    def p1(i, c):
        gs = [2 + i * U1 + k for k in range(U1)]
        for g in gs:
            wqa_cp(g).wait()
        per = G * U1 // (G - 2)
        todo = [(i * per + k, rows) for k in range(per)
                for rows in _split(D, (2 * B * U1 - 2) // per)]
        for g in gs:
            for b in range(B):
                for u in range(2):
                    qproj(0, g, b, u)
                    if todo:
                        n, rows = todo.pop(0)
                        w_cp(wqb_h, WQB, n, rows, wq_sem.at[G + n]).start(priority=SMALL)
        return c
    lax.fori_loop(0, (G - 2) // U1, p1, 0)

    xb_cp.wait()

    def p2(b, c):
        wait_filled(w_v.at[WQB + b], wq_sem.at[G + b])
        ka_cp(b).wait()
        wait_filled(va_buf(b, 0, G * SK), va_sem)
        row = pl.multiple_of(b * SQ, 16)
        todo = list(zip(_split(G * SK, N2), _split(VT * SK, N2)))
        wtodo = _split(D, NW)

        def trickle():
            if todo:
                rows, rows_b = todo.pop(0)

                @pl.when(b + 1 < B)
                def _():
                    dst = va_buf(b + 1, rows.start, rows.size)
                    copy(va_h.at[b + 1, rows], dst, va_sem).start(priority=SMALL)

                @pl.when(b + 1 == B)
                def _():
                    vb_first(b + 1 - B, rows_b).start(priority=SMALL)

        s, p = {}, {}
        for i in range(-2, H):
            h = i + 2
            if h < H:
                qproj(1, b, h // 2, h % 2)
                if wtodo:
                    w_cp(woa_h, WOA, b, wtodo.pop(0), wo_sem.at[0]).start(priority=SMALL)
                q = q_v[0][h // 2, b, h % 2 * SQ:(h % 2 + 1) * SQ]
                s[h] = scores(q, lambda r, n: ka_buf(b, h // 2 * SK + r, n)[...], trickle)
            if 0 <= i + 1 < H:
                p[i + 1] = _softmax(s[i + 1])
            if i >= 0:
                vrows = _ds((b % 2 * G + i // 2) * SK, SK, SK)
                store_pv(p[i], lambda cols: kv_v[B + 6, vrows, cols], i, row, trickle)
        assert not todo and not wtodo
        return c
    lax.fori_loop(0, B, p2, 0)

    wait_filled(w_v.at[pl.ds(WOA, G)], wo_sem.at[0])
    for b in (2, 3):
        for cp in kvb_early(b):
            cp.start(priority=BULK)
    n3 = (NT - 1) // U3

    def p3(i, c):
        todo = [(i * (G // n3) + j, rows) for j in range(G // n3) for rows in _split(D, N3)]
        done = None
        for u in range(U3):
            t = i * U3 + u
            acc = [None, None]
            for k in range(2 * G - (u == U3 - 1)):
                g, r = k // 2, k % 2
                part = oproj(WOA, t, g, pl.ds(r * HALF, HALF))
                acc[r] = part if acc[r] is None else acc[r] + part
                if todo and k >= 3:
                    n, rows = todo.pop(0)
                    w_cp(wob_h, WOB, n, rows, wo_sem.at[1]).start(priority=SMALL)
                if done is not None:
                    acc_v[t - 1] = done
                    done = None
            done = jnp.concatenate(acc, axis=0)
        acc_v[i * U3 + U3 - 1, 0:HALF, :] = acc[0]
        part_v[_ds(i * HALF, HALF, 8), :] = acc[1]
        assert not todo
        return c
    lax.fori_loop(0, n3, p3, 0)

    def attend_b(b, late):
        row = pl.multiple_of(T + b * SQ, 16)
        todo = _split(VT * SK, N5 if late else N4)
        bulk = []
        if not late:
            pl.when(b == 1)(lambda: wait_filled(w_v.at[pl.ds(WOB, G)], wo_sem.at[1]))
            for cp in kvb_early(b):
                cp.wait()
            bulk = [(b + 4 < LATE, cp) for cp in kvb_early(jnp.minimum(b + 4, LATE - 1))]
            bulk += [(b == LATE - 4, cp) for n in range(LATE, B) for j in range(NCH)
                     for cp in kvb_late(n, j)]
        vb_first(b, _heads(0, VT)).wait()

        def trickle():
            if bulk:
                cond, cp = bulk.pop(0)
                pl.when(cond)(lambda: cp.start(priority=BULK))
            if todo:
                piece = vb_first(jnp.minimum(b + 1, B - 1), todo.pop(0))
                if late:
                    pl.when(b + 1 < B)(lambda: piece.start(priority=SMALL))
                else:
                    piece.start(priority=SMALL)

        def finish_previous_tile():
            t1 = NT - 2 + b
            if late:
                done = part_v[...] + oproj(WOB, t1, G - 1)
            else:
                w0 = jnp.where(b >= 2, WOB, WOA)
                r0 = pl.multiple_of(jnp.where(b == 0, HALF, 0), 16)
                t0 = jnp.where(b == 0, U3 - 1, t1)
                done = part_v[...] + jnp.concatenate(
                    [oproj(w0, t0, G - 1, pl.ds(r0, HALF)),
                     oproj(w0, t1, G - 1, pl.ds(HALF, HALF))], axis=0)
            t = jnp.maximum(b - 2, 0)
            both = jnp.concatenate([acc_v[t, D - PAD:D, :], done], axis=0)
            out_v[_tile(t), D - PAD:2 * D] = both.T.astype(BF)
            if not late:
                acc_v[jnp.minimum(t0, NT), pl.ds(r0, HALF), :] = done[0:HALF]
                acc_v[jnp.minimum(t1, NT), HALF:D, :] = done[HALF:D]

        s, p = {}, {}
        acc = None
        for i in range(-LAG, H):
            h = i + LAG
            if late and h in KCUT[:-1]:
                for cp in kvb_late(b, KCUT.index(h)):
                    cp.wait()
                if h == KCUT[-2]:
                    def send(_, carry):
                        out_cp(0).start()
                        out_cp(1).start()
                        return carry
                    lax.fori_loop(0, jnp.where(b == B - 1, 1, 0), send, 0)
            if 0 <= i + 1 < H:
                p[i + 1] = _softmax(s[i + 1])
            if i >= 0:
                store_pv(p[i], lambda cols: kv_v[B + b, _heads(i, i + 1), cols], i, row, trickle)
            if h < H:
                q = q_v[1][h // 2, b, h % 2 * SQ:(h % 2 + 1) * SQ]
                s[h] = scores(q, lambda r, n: kv_v[b, pl.ds(h * SK + r, n)], trickle)
            if i == 1:
                finish_previous_tile()
            if i == 5:
                t = jnp.minimum(b, NT - 1)
                out_v[_tile(t), 0:D - PAD] = acc_v[t, 0:D - PAD, :].T.astype(BF)
            if i > 0 and i % 2 == 0:
                w0 = WOB if late else jnp.where(b >= 1, WOB, WOA)
                part = oproj(w0, NT - 1 + b, i // 2 - 1)
                acc = part if acc is None else acc + part
        assert not todo and not bulk
        part_v[...] = acc

    def p4a(b, c):
        attend_b(b, False)
        return c
    lax.fori_loop(0, LATE, p4a, 0)

    def p4b(b, c):
        attend_b(b, True)
        return c
    lax.fori_loop(LATE, B, p4b, 0)

    head = jnp.concatenate([acc_v[NT - 1, D - PAD:D, :], part_v[...]], axis=0).T
    w_last = jnp.concatenate([jnp.zeros((PAD, GW), BF), w_v[WOB + G - 1]], axis=0)
    for j in range(2):
        cols = slice(2 * j * TT, 2 * (j + 1) * TT)
        last = head[:, cols] + _dot_nt(o_v[G - 1][_tile(2 * NT - 1), :], w_last[cols])
        out_v[_tile(NT - 1), pl.ds(D - PAD + cols.start, 2 * TT)] = last.astype(BF)
        out_cp(2 + j).start()
    for i in range(4):
        out_cp(i).wait()


@jax.jit
def pallas_concat_heads__gqa_block_cached__mha_block_cached__near_ridge_kernel(
    A_x: jax.Array,
    A_k_cache: jax.Array,
    A_v_cache: jax.Array,
    A_wq: jax.Array,
    A_wo: jax.Array,
    B_x: jax.Array,
    B_k_cache: jax.Array,
    B_v_cache: jax.Array,
    B_wq: jax.Array,
    B_wo: jax.Array,
):
    dma = pltpu.SemaphoreType.DMA
    out = pl.pallas_call(
        _kernel,
        out_shape=jax.ShapeDtypeStruct((T, 2 * D), BF),
        in_specs=[pl.BlockSpec(memory_space=pl.ANY)] * 10,
        out_specs=pl.BlockSpec(memory_space=pl.ANY),
        scratch_shapes=[
            pltpu.VMEM((2, T, D), BF),
            pltpu.VMEM((4 * G, D, GW), BF),
            pltpu.VMEM((2 * B, H * SK, DH), BF),
            [pltpu.VMEM((G, B, 2 * SQ, DH), BF)] * 2,
            [pltpu.VMEM((2 * T, GW), BF)] * G,
            pltpu.VMEM((NT + 1, D, TT), F32),
            pltpu.VMEM((D, TT), F32),
            pltpu.VMEM((T, 2 * D), BF),
            dma((len(XCUT) + 2,)),
            dma((2 * G,)),
            dma((2,)),
            dma((B,)),
            dma(()),
            dma((LATE + (B - LATE) * NCH,)),
            dma((2,)),
            dma((4,)),
        ],
        compiler_params=pltpu.CompilerParams(
            vmem_limit_bytes=120 * 1024 * 1024,
            disable_bounds_checks=True,
            disable_semaphore_checks=True,
        ),
    )(
        A_x.reshape(T, D), A_k_cache.reshape(B, G * SK, DH), A_v_cache.reshape(B, G * SK, DH),
        A_wq, A_wo.T,
        B_x.reshape(T, D), B_k_cache.reshape(B, H * SK, DH), B_v_cache.reshape(B, H * SK, DH),
        B_wq, B_wo.T,
    )
    return out.reshape(B, SQ, 2 * D)
```
